```python
import os as _os
_os.environ.setdefault("JAX_PLATFORMS", "cpu")
import jax
import jax.numpy as jnp

def _softmax(x, axis=-1):
    return jax.nn.softmax(x, axis=axis)
def _gelu(x):
    return jax.nn.gelu(x, approximate=True)
def _silu(x):
    return jax.nn.silu(x)
def _sigmoid(x):
    return jax.nn.sigmoid(x)
def _layernorm(x, axis=-1, eps=1e-5):
    m = jnp.mean(x, axis=axis, keepdims=True)
    v = jnp.var(x, axis=axis, keepdims=True)
    return (x - m) / jnp.sqrt(v + eps)
def _scatter_add(tgt, idx, src, axis=0):
    return tgt.at[idx].add(src)
def _segment_sum(src, seg, n):
    return jax.ops.segment_sum(src, seg, n)
class _Rng:
    def __init__(self, key):
        self._k = key
    def _next(self):
        self._k, sub = jax.random.split(self._k)
        return sub
    def normal(self, shape):
        return jax.random.normal(self._next(), shape, dtype=jnp.bfloat16)
    def randint(self, lo, hi, shape):
        return jax.random.randint(self._next(), shape, lo, hi, dtype=jnp.int32)
    def uniform(self, shape, lo=0.0, hi=1.0):
        return jax.random.uniform(self._next(), shape, jnp.bfloat16, lo, hi)
    def permutation(self, n):
        return jax.random.permutation(self._next(), n)


kernel_name = 'standalone__gqa_block_cached__near_ridge'

def setup_inputs():
    _rng = _Rng(jax.random.key(int.from_bytes(__import__("os").urandom(4), "little")))
    _w = (lambda a: (lambda t: t.astype(jnp.bfloat16) if jnp.issubdtype(t.dtype, jnp.floating) else t)(jnp.asarray(a)))
    B, Sq, D = 8, 96, 640
    Hq, Hkv, Sk, Dh = 32, 32, 512, 128
    assert Hq % Hkv == 0, (Hq, Hkv)
    return {
        "x": _w((lambda *s: _rng.normal(s) * 0.2)(B, Sq, D)),
        "k_cache": _w((lambda *s: _rng.normal(s) * 3.2)(B, Hkv, Sk, Dh)),
        "v_cache": _w((lambda *s: _rng.normal(s) * 0.05)(B, Hkv, Sk, Dh)),
        "wq": _w((lambda *s: _rng.normal(s) * 0.2)(D, Hq * Dh) * (D ** -0.5)),
        "wo": _w((lambda *s: _rng.normal(s) * 0.05)(Hq * Dh, D) * ((Hq * Dh) ** -0.5)),
    }

def reference(x, k_cache, v_cache, wq, wo):
    B, Sq, D = x.shape
    Hq, Dh = 32, 128
    Hkv = k_cache.shape[1]
    rep = Hq // Hkv
    q = (lambda x, *d: x.transpose(*d))((x @ wq).reshape(B, Sq, Hq, Dh), 0, 2, 1, 3)
    k = jnp.repeat(k_cache, rep, axis=1)
    v = jnp.repeat(v_cache, rep, axis=1)
    scores = jnp.einsum("bhqd,bhkd->bhqk", q, k) * (Dh ** -0.5)
    p = _softmax(scores, axis=-1)
    o = jnp.einsum("bhqk,bhkd->bhqd", p, v)
    return (lambda x, *d: x.transpose(*d))(o, 0, 2, 1, 3).reshape(B, Sq, Hq * Dh) @ wo
```

```python
import functools
import jax
import jax.numpy as jnp
import jax.experimental.pallas as pl
import jax.experimental.pallas.tpu as pltpu

B, SQ, D = 8, 96, 640
H, SK, DH = 32, 512, 128
M = B * SQ
LOG2E = 1.4426950408889634
U32 = jnp.uint32
BF = jnp.bfloat16
F32 = jnp.float32
NT = (((1,), (1,)), ((), ()))
R = SQ // 2


def bf(x):
    return pltpu.bitcast(x, BF)


def make_v3(NB=4, order=('qk', 'qp', 'pv', 'op'), flags=None, vmem_mb=100, nobounds=True, sscr=False, group=8):
    SC = DH ** -0.5 * LOG2E

    def kernel(x_hbm, k_hbm, v_hbm, wq_hbm, wo_hbm, o_hbm,
               xbuf, wqbuf, kbuf, vbuf, wobuf, q_scr, o_scr, acc, obuf, sem_x, sem_wq, sem_k, sem_v, sem_wo, sem_o):
        xh = x_hbm.bitcast(U32); kh = k_hbm.bitcast(U32); vh = v_hbm.bitcast(U32)
        wqh = wq_hbm.bitcast(U32); woh = wo_hbm.bitcast(U32)
        q32 = q_scr.bitcast(U32); o32 = o_scr.bitcast(U32)

        def cp_x():
            return pltpu.make_async_copy(xh, xbuf, sem_x.at[0])
        def cp_wq(h):
            s = h % NB
            return pltpu.make_async_copy(wqh.at[:, pl.ds(pl.multiple_of(h * DH, DH), DH)], wqbuf.at[s], sem_wq.at[s])
        def cp_wo(h):
            s = h % NB
            return pltpu.make_async_copy(woh.at[pl.ds(pl.multiple_of(h * (DH // 2), DH // 2), DH // 2), :], wobuf.at[s], sem_wo.at[s])
        def cp_k(h):
            s = h % NB
            return pltpu.make_async_copy(kh.at[:, h], kbuf.at[s], sem_k.at[s])
        def cp_v(h):
            s = h % NB
            return pltpu.make_async_copy(vh.at[:, h], vbuf.at[s], sem_v.at[s])

        def qproj(h, b):
            q = jnp.dot(bf(xbuf[b * R:(b + 1) * R, :]), bf(wqbuf[h % NB]), preferred_element_type=F32)
            q_scr[h % 2, b * SQ:(b + 1) * SQ, :] = (q * SC).astype(BF)

        def oproj(h, b):
            o = bf(o32[(h + 2) % 2, b * R:(b + 1) * R, :])
            r = jnp.dot(o, bf(wobuf[(h + NB) % NB]), preferred_element_type=F32)
            acc[b * SQ:(b + 1) * SQ, :] += r

        def qk(h, b):
            q = bf(q32[h % 2, b * R:(b + 1) * R, :])
            k = bf(kbuf[h % NB, b])
            return jax.lax.dot_general(q, k, NT, preferred_element_type=F32)

        def softmax(s):
            m = jnp.max(s, axis=-1, keepdims=True)
            p = jnp.exp2(s - m)
            l = jnp.sum(p, axis=-1, keepdims=True)
            r = pl.reciprocal(l, approx=True)
            r = r * (2.0 - l * r)
            return p.astype(BF), r

        def pv(h, b, s):
            p, r = softmax(s)
            v = bf(vbuf[h % NB, b])
            o = jnp.dot(p, v, preferred_element_type=F32)
            o_scr[h % 2, b * SQ:(b + 1) * SQ, :] = (o * r).astype(BF)

        cp_x().start()
        cp_wq(0).start()
        for h in range(NB):
            cp_k(h).start()
            if h + 1 < NB:
                cp_wq(h + 1).start()
            cp_v(h).start()
            if h < NB - 1:
                cp_wo(h).start()
        acc[...] = jnp.zeros(acc.shape, F32)
        o_scr[1] = jnp.zeros(o_scr.shape[1:], BF)
        wobuf[NB - 1] = jnp.zeros(wobuf.shape[1:], U32)
        cp_x().wait()
        cp_wq(0).wait()
        for b in range(B):
            qproj(0, b)
        cp_wq(NB).start()

        def body(h, last):
            cp_k(h).wait()
            cp_v(h).wait()
            if not last:
                cp_wq(h + 1).wait()
            if last:
                cp_wo(h - 1).wait()
            else:
                @pl.when(h >= 1)
                def _():
                    cp_wo(h - 1).wait()
            ss = {}
            for g0 in range(0, B, group):
              bs = range(g0, g0 + group)
              for ph in order:
                if ph == 'qk':
                    for b in bs:
                        ss[b] = qk(h, b)
                    if not last and g0 + group == B:
                        @pl.when(h + NB < H)
                        def _():
                            cp_k(h + NB).start()
                elif ph == 'qp' and not last:
                    for b in bs:
                        qproj(h + 1, b)
                    if g0 + group == B:
                        @pl.when(h + 1 + NB < H)
                        def _():
                            cp_wq(h + 1 + NB).start()
                elif ph == 'pv':
                    for b in bs:
                        pv(h, b, ss[b])
                    if not last and g0 + group == B:
                        @pl.when(h + NB < H)
                        def _():
                            cp_v(h + NB).start()
                elif ph == 'op':
                    for b in bs:
                        oproj(h - 1, b)
                    if not last and g0 + group == B:
                        @pl.when(h - 1 + NB < H)
                        def _():
                            cp_wo(h - 1 + NB).start()

        def loop(h, c):
            body(h, False)
            return c
        jax.lax.fori_loop(0, H - 1, loop, 0)
        body(H - 1, True)
        cp_wo(H - 1).wait()
        for b in range(B):
            o = bf(o32[(H - 1) % 2, b * R:(b + 1) * R, :])
            r = jnp.dot(o, bf(wobuf[(H - 1) % NB]), preferred_element_type=F32)
            obuf[b * SQ:(b + 1) * SQ, :] = (acc[b * SQ:(b + 1) * SQ, :] + r).astype(BF)
        c = pltpu.make_async_copy(obuf, o_hbm, sem_o.at[0])
        c.start(); c.wait()

    def fn(x, k_cache, v_cache, wq, wo):
        any_spec = pl.BlockSpec(memory_space=pl.ANY)
        out = pl.pallas_call(
            kernel,
            in_specs=[any_spec] * 5,
            out_specs=any_spec,
            out_shape=jax.ShapeDtypeStruct((M, D), BF),
            scratch_shapes=[
                pltpu.VMEM((M // 2, D), U32),
                pltpu.VMEM((NB, D // 2, DH), U32),
                pltpu.VMEM((NB, B, SK // 2, DH), U32),
                pltpu.VMEM((NB, B, SK // 2, DH), U32),
                pltpu.VMEM((NB, DH // 2, D), U32),
                pltpu.VMEM((2, M, DH), BF),
                pltpu.VMEM((2, M, DH), BF),
                pltpu.VMEM((M, D), F32),
                pltpu.VMEM((M, D), BF),
                pltpu.SemaphoreType.DMA((1,)),
                pltpu.SemaphoreType.DMA((NB,)),
                pltpu.SemaphoreType.DMA((NB,)),
                pltpu.SemaphoreType.DMA((NB,)),
                pltpu.SemaphoreType.DMA((NB,)),
                pltpu.SemaphoreType.DMA((1,)),
            ],
            compiler_params=pltpu.CompilerParams(vmem_limit_bytes=vmem_mb << 20, flags=flags, disable_bounds_checks=nobounds),
        )(x.reshape(M, D), k_cache, v_cache, wq, wo)
        return out.reshape(B, SQ, D)
    return jax.jit(fn)


_FN = make_v3()


@jax.jit
def pallas_standalone__gqa_block_cached__near_ridge_kernel(x, k_cache, v_cache, wq, wo):
    return _FN(x, k_cache, v_cache, wq, wo)
```

```python
import jax
import jax.numpy as jnp
import jax.experimental.pallas as pl
import jax.experimental.pallas.tpu as pltpu

B, SQ, D = 8, 96, 640
H, SK, DH = 32, 512, 128
M = B * SQ
U32, BF, F32 = jnp.uint32, jnp.bfloat16, jnp.float32
NT_DIMS = (((1,), (1,)), ((), ()))

Q_SCALE = DH ** -0.5 * 1.4426950408889634

LOOKAHEAD = 4
PREFETCH = 2
SLOTS = PREFETCH + 1
WSEM = PREFETCH + LOOKAHEAD
CHUNK = 64
NCHUNK = SK // 2 // CHUNK
BATCH_ORDER = (0, 4, 1, 5, 2, 6, 3, 7)
CHUNKS = tuple((b, c) for c in range(NCHUNK) for b in BATCH_ORDER)
LAST = H - 1
HALF = B // 2


def _bf16(words):
    return pltpu.bitcast(words, BF)


def _kernel(x_hbm, k_hbm, v_hbm, wq_hbm, wo_hbm, out_hbm,
           x_buf, wq_buf, kv_buf, wo_buf, q_buf, o_buf, acc, out_buf,
           sem_x, sem_wq, sem_wo, sem_k, sem_v, sem_vlast, sem_out):
    x32, k32, v32, wq32, wo32 = (
        r.bitcast(U32) for r in (x_hbm, k_hbm, v_hbm, wq_hbm, wo_hbm))
    k_buf, v_buf = kv_buf.at[0], kv_buf.at[1]

    def rows(b):
        return slice(b * SQ, (b + 1) * SQ)

    def wq_copy(h):
        cols = pl.ds(pl.multiple_of(h * DH, DH), DH)
        return pltpu.make_async_copy(wq32.at[:, cols], wq_buf.at[h], sem_wq.at[h % WSEM])

    def wo_rows(h):
        return pl.ds(pl.multiple_of(h * (DH // 2), DH // 2), DH // 2)

    def wo_copy(h):
        return pltpu.make_async_copy(
            wo32.at[wo_rows(h), :], wo_buf.at[wo_rows(h), :], sem_wo.at[h % WSEM])

    def k_copy(h, b, c):
        r = pl.ds(c * CHUNK, CHUNK)
        return pltpu.make_async_copy(
            k32.at[b, h, r], k_buf.at[h % SLOTS, b, r], sem_k.at[h % SLOTS])

    def v_copy(h, b, c, sem):
        r = pl.ds(c * CHUNK, CHUNK)
        return pltpu.make_async_copy(v32.at[b, h, r], v_buf.at[h % SLOTS, b, r], sem)

    def fill(dst, sem):
        pltpu.make_async_copy(dst, dst, sem).wait()

    def start_kv(h, chunks=CHUNKS):
        for b, c in chunks:
            k_copy(h, b, c).start(priority=0)
            v_copy(h, b, c, sem_v.at[h % SLOTS]).start(priority=1)

    def wait_k(h):
        fill(k_buf.at[h % SLOTS], sem_k.at[h % SLOTS])

    def wait_v(h):
        fill(v_buf.at[h % SLOTS], sem_v.at[h % SLOTS])

    def q_proj(h, b):
        xb = _bf16(x_buf[b * SQ // 2:(b + 1) * SQ // 2, :])
        q = jnp.dot(xb, _bf16(wq_buf[h]), preferred_element_type=F32)
        q_buf[h, rows(b), :] = (q * Q_SCALE).astype(BF)

    def scores(h, b):
        s = jax.lax.dot_general(q_buf[h, rows(b), :], _bf16(k_buf[h % SLOTS, b]),
                                NT_DIMS, preferred_element_type=F32)
        p = jnp.exp2(s - jnp.max(s, axis=-1, keepdims=True))
        l = jnp.sum(p, axis=-1, keepdims=True)
        r = pl.reciprocal(l, approx=True)
        return p.astype(BF), r * (2.0 - l * r)

    def attend(h, b, pr):
        p, r = pr
        o = jnp.dot(p, _bf16(v_buf[h % SLOTS, b]), preferred_element_type=F32)
        o_buf[h % 2, rows(b), :] = (o * r).astype(BF)

    def o_proj(h, b):
        acc[rows(b), :] += jnp.dot(o_buf[h % 2, rows(b), :], _bf16(wo_buf[wo_rows(h), :]),
                                   preferred_element_type=F32)

    def out_copy(b):
        r = pl.ds(b * SQ, SQ)
        return pltpu.make_async_copy(out_buf.at[r], out_hbm.at[r], sem_out.at[0])

    def o_proj_last(b):
        o = o_buf[LAST % 2, rows(b), :]
        for j in range(D // 128):
            cols = slice(j * 128, (j + 1) * 128)
            w = _bf16(wo_buf[LAST * DH // 2:(LAST + 1) * DH // 2, cols])
            y = acc[rows(b), cols] + jnp.dot(o, w, preferred_element_type=F32)
            out_buf[rows(b), cols] = y.astype(BF)
        out_copy(b).start(priority=1)

    for i in range(2):
        r = pl.ds(i * M // 4, M // 4)
        pltpu.make_async_copy(x32.at[r], x_buf.at[r], sem_x.at[0]).start(priority=i)
    for h in range(LOOKAHEAD):
        wq_copy(h).start(priority=h % 2)
    for h in range(PREFETCH):
        wq_copy(h + LOOKAHEAD).start(priority=0)
        wo_copy(h).start(priority=1)
        start_kv(h)
    acc[...] = jnp.zeros(acc.shape, F32)
    fill(x_buf, sem_x.at[0])
    for h in range(LOOKAHEAD):
        wq_copy(h).wait()
    for h in range(LOOKAHEAD):
        for b in range(B):
            q_proj(h, b)

    def step(h, carry):
        wq_copy(h + LOOKAHEAD).wait()
        wo_copy(h).wait()
        wait_v(h)
        wait_k(h)
        nxt = h + PREFETCH

        @pl.when(nxt + LOOKAHEAD < H)
        def _():
            wq_copy(jnp.minimum(nxt + LOOKAHEAD, LAST)).start(priority=0)
        wo_copy(nxt).start(priority=1)

        pr = [scores(h, b) for b in range(B)]
        per = len(CHUNKS) // HALF
        for b in range(HALF):
            q_proj(h + LOOKAHEAD, b)
            start_kv(nxt, CHUNKS[b * per:(b + 1) * per])
        for b in range(B):
            attend(h, b, pr[b])
        for b in range(HALF, B):
            q_proj(h + LOOKAHEAD, b)
        for b in range(B):
            o_proj(h, b)
        return carry

    jax.lax.fori_loop(0, H - LOOKAHEAD, step, 0)

    h0, h1, h2, h3 = range(H - LOOKAHEAD, H)

    def all_scores(h):
        return [scores(h, b) for b in range(B)]

    def all_attend(h, pr, bs=range(B)):
        for b in bs:
            attend(h, b, pr[b])

    def all_o_proj(h):
        for b in range(B):
            o_proj(h, b)

    wait_k(h0)
    pr0 = all_scores(h0)

    wait_v(h0); wo_copy(h0).wait(); wait_k(h1)
    all_attend(h0, pr0)
    wo_copy(h2).start(priority=1)
    start_kv(h2)
    pr1 = all_scores(h1)
    all_o_proj(h0)

    wait_v(h1); wo_copy(h1).wait()
    all_attend(h1, pr1)
    for b, c in CHUNKS:
        k_copy(h3, b, c).start(priority=1)
    all_o_proj(h1)

    wait_k(h2)
    pr2 = all_scores(h2)
    for b in range(B):
        for c in range(NCHUNK):
            v_copy(h3, b, c, sem_vlast.at[b // HALF]).start(priority=1)
    wo_copy(h3).start(priority=1)

    wait_v(h2); wo_copy(h2).wait()
    all_attend(h2, pr2)
    all_o_proj(h2)

    wait_k(h3)
    pr3 = all_scores(h3)

    for half in range(2):
        bs = range(half * HALF, (half + 1) * HALF)
        fill(v_buf.at[h3 % SLOTS, pl.ds(half * HALF, HALF)], sem_vlast.at[half])
        if half == 0:
            wo_copy(h3).wait()
        all_attend(h3, pr3, bs)
        for b in bs:
            o_proj_last(b)

    fill(out_buf, sem_out.at[0])


@jax.jit
def pallas_standalone__gqa_block_cached__near_ridge_kernel(x, k_cache, v_cache, wq, wo):
    hbm = pl.BlockSpec(memory_space=pl.ANY)
    out = pl.pallas_call(
        _kernel,
        in_specs=[hbm] * 5,
        out_specs=hbm,
        out_shape=jax.ShapeDtypeStruct((M, D), BF),
        scratch_shapes=[
            pltpu.VMEM((M // 2, D), U32),
            pltpu.VMEM((H, D // 2, DH), U32),
            pltpu.VMEM((2, SLOTS, B, SK // 2, DH), U32),
            pltpu.VMEM((H * DH // 2, D), U32),
            pltpu.VMEM((H, M, DH), BF),
            pltpu.VMEM((2, M, DH), BF),
            pltpu.VMEM((M, D), F32),
            pltpu.VMEM((M, D), BF),
            pltpu.SemaphoreType.DMA((1,)),
            pltpu.SemaphoreType.DMA((WSEM,)),
            pltpu.SemaphoreType.DMA((WSEM,)),
            pltpu.SemaphoreType.DMA((SLOTS,)),
            pltpu.SemaphoreType.DMA((SLOTS,)),
            pltpu.SemaphoreType.DMA((2,)),
            pltpu.SemaphoreType.DMA((1,)),
        ],
        compiler_params=pltpu.CompilerParams(
            vmem_limit_bytes=64 * 1024 * 1024,
            disable_bounds_checks=True,
            disable_semaphore_checks=True,
        ),
    )(x.reshape(M, D), k_cache, v_cache, wq, wo)
    return out.reshape(B, SQ, D)
```

```python
import jax
import jax.numpy as jnp
import jax.experimental.pallas as pl
import jax.experimental.pallas.tpu as pltpu

B, SQ, D = 8, 96, 640
H, SK, DH = 32, 512, 128
M = B * SQ
LANES = 128
U32, BF, F32 = jnp.uint32, jnp.bfloat16, jnp.float32
NT_DIMS = (((1,), (1,)), ((), ()))

Q_SCALE = DH ** -0.5 * 1.4426950408889634

LOOKAHEAD = 4
PREFETCH = 2
SLOTS = PREFETCH + 1
WSEM = PREFETCH + LOOKAHEAD
CHUNK = 64
NCHUNK = SK // 2 // CHUNK
CHUNKS = tuple((b, c) for c in range(NCHUNK) for b in (0, 4, 1, 5, 2, 6, 3, 7))
LAST = H - 1
HALF = B // 2
LAST_GROUPS = ((0, 4), (4, 6), (6, 8))


def _bf16(words):
    return pltpu.bitcast(words, BF)


def _kernel(x_hbm, k_hbm, v_hbm, wq_hbm, wo_hbm, out_hbm,
            x_buf, wq_buf, kv_buf, wo_buf, q_buf, o_buf, acc, out_buf,
            sem_x, sem_wq, sem_wo, sem_k, sem_v, sem_vlast, sem_out):
    x32, k32, v32, wq32, wo32 = (
        r.bitcast(U32) for r in (x_hbm, k_hbm, v_hbm, wq_hbm, wo_hbm))
    k_buf, v_buf = kv_buf.at[0], kv_buf.at[1]

    def rows(b):
        return slice(b * SQ, (b + 1) * SQ)

    def wq_copy(h):
        cols = pl.ds(pl.multiple_of(h * DH, DH), DH)
        return pltpu.make_async_copy(wq32.at[:, cols], wq_buf.at[h], sem_wq.at[h % WSEM])

    def wo_rows(h):
        return pl.ds(pl.multiple_of(h * (DH // 2), DH // 2), DH // 2)

    def wo_copy(h):
        return pltpu.make_async_copy(
            wo32.at[wo_rows(h), :], wo_buf.at[wo_rows(h), :], sem_wo.at[h % WSEM])

    def k_copy(h, b, c):
        r = pl.ds(c * CHUNK, CHUNK)
        return pltpu.make_async_copy(
            k32.at[b, h, r], k_buf.at[h % SLOTS, b, r], sem_k.at[h % SLOTS])

    def v_copy(h, b, c, sem):
        r = pl.ds(c * CHUNK, CHUNK)
        return pltpu.make_async_copy(v32.at[b, h, r], v_buf.at[h % SLOTS, b, r], sem)

    def out_copy(b):
        r = pl.ds(b * SQ, SQ)
        return pltpu.make_async_copy(out_buf.at[r], out_hbm.at[r], sem_out.at[0])

    def wait_filled(buf, sem):
        pltpu.make_async_copy(buf, buf, sem).wait()

    def start_kv(h, chunks=CHUNKS):
        for b, c in chunks:
            k_copy(h, b, c).start(priority=0)
            v_copy(h, b, c, sem_v.at[h % SLOTS]).start(priority=1)

    def wait_k(h):
        wait_filled(k_buf.at[h % SLOTS], sem_k.at[h % SLOTS])

    def wait_v(h):
        wait_filled(v_buf.at[h % SLOTS], sem_v.at[h % SLOTS])

    def q_proj(h, b):
        xb = _bf16(x_buf[b * SQ // 2:(b + 1) * SQ // 2, :])
        q = jnp.dot(xb, _bf16(wq_buf[h]), preferred_element_type=F32)
        q_buf[h, rows(b), :] = (q * Q_SCALE).astype(BF)

    def scores(h, b):
        s = jax.lax.dot_general(q_buf[h, rows(b), :], _bf16(k_buf[h % SLOTS, b]),
                                NT_DIMS, preferred_element_type=F32)
        p = jnp.exp2(s - jnp.max(s, axis=-1, keepdims=True))
        l = jnp.sum(p, axis=-1, keepdims=True)
        r = pl.reciprocal(l, approx=True)
        return p.astype(BF), r * (2.0 - l * r)

    def attend(h, b, pr):
        p, r = pr
        o = jnp.dot(p, _bf16(v_buf[h % SLOTS, b]), preferred_element_type=F32)
        o_buf[h % 2, rows(b), :] = (o * r).astype(BF)

    def o_proj(h, b):
        acc[rows(b), :] += jnp.dot(o_buf[h % 2, rows(b), :], _bf16(wo_buf[wo_rows(h), :]),
                                   preferred_element_type=F32)

    def all_scores(h):
        return [scores(h, b) for b in range(B)]

    def all_attend(h, pr):
        for b in range(B):
            attend(h, b, pr[b])

    def all_o_proj(h):
        for b in range(B):
            o_proj(h, b)

    def attend_tiled(h, b, pr):
        p, r = pr
        o = None
        for j in range(SK // LANES):
            v = _bf16(v_buf[h % SLOTS, b, j * LANES // 2:(j + 1) * LANES // 2, :])
            t = jnp.dot(p[:, j * LANES:(j + 1) * LANES], v, preferred_element_type=F32)
            o = t if o is None else o + t
        o_buf[h % 2, rows(b), :] = (o * r).astype(BF)

    def o_proj_last(b):
        o = o_buf[LAST % 2, rows(b), :]
        for j in range(D // LANES):
            cols = slice(j * LANES, (j + 1) * LANES)
            w = _bf16(wo_buf[LAST * DH // 2:(LAST + 1) * DH // 2, cols])
            y = acc[rows(b), cols] + jnp.dot(o, w, preferred_element_type=F32)
            out_buf[rows(b), cols] = y.astype(BF)
        out_copy(b).start(priority=1)

    def start_head(h):
        wq_copy(h + LOOKAHEAD).start(priority=0)
        wo_copy(h).start(priority=1)
        start_kv(h)

    for i in range(2):
        r = pl.ds(i * M // 4, M // 4)
        pltpu.make_async_copy(x32.at[r], x_buf.at[r], sem_x.at[0]).start(priority=i)
    for h in range(LOOKAHEAD):
        wq_copy(h).start(priority=h % 2)
    start_head(0)
    acc[...] = jnp.zeros(acc.shape, F32)
    wait_filled(x_buf, sem_x.at[0])
    wq_copy(0).wait()
    for b in range(B):
        q_proj(0, b)
    for h in range(1, PREFETCH):
        start_head(h)
    for h in range(1, LOOKAHEAD):
        wq_copy(h).wait()
    for h in range(1, LOOKAHEAD):
        for b in range(B):
            q_proj(h, b)

    def step(h, carry):
        wq_copy(h + LOOKAHEAD).wait()
        wo_copy(h).wait()
        wait_v(h)
        wait_k(h)
        nxt = h + PREFETCH

        @pl.when(nxt + LOOKAHEAD < H)
        def _():
            wq_copy(jnp.minimum(nxt + LOOKAHEAD, LAST)).start(priority=0)
        wo_copy(nxt).start(priority=1)

        pr = all_scores(h)
        n = len(CHUNKS) // HALF
        for b in range(HALF):
            q_proj(h + LOOKAHEAD, b)
            start_kv(nxt, CHUNKS[b * n:(b + 1) * n])
        all_attend(h, pr)
        for b in range(HALF, B):
            q_proj(h + LOOKAHEAD, b)
        all_o_proj(h)
        return carry

    jax.lax.fori_loop(0, H - LOOKAHEAD, step, 0)

    h0, h1, h2, h3 = range(H - LOOKAHEAD, H)

    wait_k(h0)
    pr0 = all_scores(h0)

    wait_v(h0)
    wo_copy(h0).wait()
    wait_k(h1)
    all_attend(h0, pr0)
    wo_copy(h2).start(priority=1)
    start_kv(h2)
    pr1 = all_scores(h1)
    all_o_proj(h0)

    wait_v(h1)
    wo_copy(h1).wait()
    all_attend(h1, pr1)
    for b, c in CHUNKS:
        k_copy(h3, b, c).start(priority=1)
    all_o_proj(h1)

    wait_k(h2)
    pr2 = all_scores(h2)
    for g, (b0, b1) in enumerate(LAST_GROUPS):
        for b in range(b0, b1):
            for c in range(NCHUNK):
                v_copy(h3, b, c, sem_vlast.at[g]).start(priority=1)
    wo_copy(h3).start(priority=1)

    wait_v(h2)
    wo_copy(h2).wait()
    all_attend(h2, pr2)
    all_o_proj(h2)

    wait_k(h3)
    pr3 = all_scores(h3)

    for g, (b0, b1) in enumerate(LAST_GROUPS):
        wait_filled(v_buf.at[h3 % SLOTS, pl.ds(b0, b1 - b0)], sem_vlast.at[g])
        if g == 0:
            wo_copy(h3).wait()
            for b in range(b0, b1):
                attend(h3, b, pr3[b])
            for b in range(b0, b1):
                o_proj_last(b)
        else:
            attend_tiled(h3, b0, pr3[b0])
            for b in range(b0, b1):
                if b + 1 < b1:
                    attend_tiled(h3, b + 1, pr3[b + 1])
                o_proj_last(b)

    wait_filled(out_buf, sem_out.at[0])


@jax.jit
def pallas_standalone__gqa_block_cached__near_ridge_kernel(
    x: jax.Array,
    k_cache: jax.Array,
    v_cache: jax.Array,
    wq: jax.Array,
    wo: jax.Array,
):
    assert x.shape == (B, SQ, D) and wq.shape == (D, H * DH) and wo.shape == (H * DH, D)
    assert k_cache.shape == v_cache.shape == (B, H, SK, DH)
    hbm = pl.BlockSpec(memory_space=pl.ANY)
    out = pl.pallas_call(
        _kernel,
        in_specs=[hbm] * 5,
        out_specs=hbm,
        out_shape=jax.ShapeDtypeStruct((M, D), BF),
        scratch_shapes=[
            pltpu.VMEM((M // 2, D), U32),
            pltpu.VMEM((H, D // 2, DH), U32),
            pltpu.VMEM((2, SLOTS, B, SK // 2, DH), U32),
            pltpu.VMEM((H * DH // 2, D), U32),
            pltpu.VMEM((H, M, DH), BF),
            pltpu.VMEM((2, M, DH), BF),
            pltpu.VMEM((M, D), F32),
            pltpu.VMEM((M, D), BF),
            pltpu.SemaphoreType.DMA((1,)),
            pltpu.SemaphoreType.DMA((WSEM,)),
            pltpu.SemaphoreType.DMA((WSEM,)),
            pltpu.SemaphoreType.DMA((SLOTS,)),
            pltpu.SemaphoreType.DMA((SLOTS,)),
            pltpu.SemaphoreType.DMA((len(LAST_GROUPS),)),
            pltpu.SemaphoreType.DMA((1,)),
        ],
        compiler_params=pltpu.CompilerParams(
            vmem_limit_bytes=64 * 1024 * 1024,
            disable_bounds_checks=True,
            disable_semaphore_checks=True,
        ),
    )(x.reshape(M, D), k_cache, v_cache, wq, wo)
    return out.reshape(B, SQ, D)
```
